```python
import jax
import jax.numpy as jnp

def _softmax(x, axis=-1):
    return jax.nn.softmax(x, axis=axis)
def _gelu(x):
    return jax.nn.gelu(x, approximate=True)
def _silu(x):
    return jax.nn.silu(x)
def _sigmoid(x):
    return jax.nn.sigmoid(x)
def _layernorm(x, axis=-1, eps=1e-5):
    m = jnp.mean(x, axis=axis, keepdims=True)
    v = jnp.var(x, axis=axis, keepdims=True)
    return (x - m) / jnp.sqrt(v + eps)
def _scatter_add(tgt, idx, src, axis=0):
    return tgt.at[idx].add(src)
def _segment_sum(src, seg, n):
    return jax.ops.segment_sum(src, seg, n)
class _Rng:
    def __init__(self, key):
        self._k = key
    def _next(self):
        self._k, sub = jax.random.split(self._k)
        return sub
    def normal(self, shape):
        return jax.random.normal(self._next(), shape, dtype=jnp.bfloat16)
    def randint(self, lo, hi, shape):
        return jax.random.randint(self._next(), shape, lo, hi, dtype=jnp.int32)
    def uniform(self, shape, lo=0.0, hi=1.0):
        return jax.random.uniform(self._next(), shape, jnp.bfloat16, lo, hi)
    def permutation(self, n):
        return jax.random.permutation(self._next(), n)


kernel_name = 'standalone__seq2seq_rnn_t_joint__speech'

def _fwd_setup_inputs():
    _rng = _Rng(jax.random.key(int.from_bytes(__import__("os").urandom(4), "little")))
    _w = (lambda a: (lambda t: t.astype(jnp.bfloat16) if jnp.issubdtype(t.dtype, jnp.floating) else t)(jnp.asarray(a)))
    B, T, D, K = 2, 4000, 256, 3
    U = 8
    sc = (1.0 / (K * D)) ** 0.5
    sd = (1.0 / D) ** 0.5
    return {
        "x": _w((lambda *s: _rng.normal(s) * 0.05)(B, T, D) * 0.5),
        "w1": _w((lambda *s: _rng.normal(s) * 0.05)(K, D, D) * sc),
        "w2": _w((lambda *s: _rng.normal(s) * 0.05)(K, D, D) * sc),
        "g": _w((lambda *s: _rng.normal(s) * 0.05)(B, U, D) * 0.5),
        "w_f": _w((lambda *s: _rng.normal(s) * 0.05)(D, D) * sd),
        "w_g": _w((lambda *s: _rng.normal(s) * 0.05)(D, D) * sd),
        "w_o": _w((lambda *s: _rng.normal(s) * 0.05)(D, D) * sd),
    }

def _fwd_reference(x, w1, w2, g, w_f, w_g, w_o):
    B, T, D = x.shape
    K = w1.shape[0]
    pad = K // 2
    xp = jnp.pad(x, ((0,0),(pad,pad),(0,0)))
    h = jnp.zeros_like(x)
    for i in range(K):
        h = h + jnp.einsum("btc,cd->btd", xp[:, i:i+T, :], w1[i])
    h = _gelu(h)[:, ::2, :]
    T1 = h.shape[1]
    hp = jnp.pad(h, ((0,0),(pad,pad),(0,0)))
    f = jnp.zeros_like(h)
    for i in range(K):
        f = f + jnp.einsum("btc,cd->btd", hp[:, i:i+T1, :], w2[i])
    f = _gelu(f)[:, ::2, :]
    fe = jnp.einsum("btd,de->bte", f, w_f)
    ge = jnp.einsum("bud,de->bue", g, w_g)
    j = jnp.tanh(fe[:, :, None, :] + ge[:, None, :, :])
    return jnp.einsum("btud,dv->btuv", j, w_o)


def setup_inputs():
    _inp = _fwd_setup_inputs()
    _gk = jax.random.fold_in(jax.random.key(int.from_bytes(__import__("os").urandom(4), "little")), 2**31 - 1)
    _shapes = [[2, 1000, 8, 256]]
    _dtypes = ['bfloat16']
    _gks = jax.random.split(_gk, len(_shapes))
    _gs = [jax.random.normal(k, s, dtype=jnp.dtype(d)) * 0.05 for k, s, d in zip(_gks, _shapes, _dtypes)]
    _inp["grad_out"] = _gs[0]
    return _inp

def reference(x, w1, w2, g, w_f, w_g, w_o, grad_out):
    _const = dict()
    def _f(*_d):
        return _fwd_reference(**{'x': _d[0], 'w1': _d[1], 'w2': _d[2], 'g': _d[3], 'w_f': _d[4], 'w_g': _d[5], 'w_o': _d[6], **_const})
    _out, _vjp = jax.vjp(_f, x, w1, w2, g, w_f, w_g, w_o)
    _grads = _vjp(grad_out)
    _out0 = jnp.asarray(_out)
    return (_out0, *[jnp.asarray(_g) for _g in _grads])
```

```python
import jax
import jax.numpy as jnp
import jax.experimental.pallas as pl
import jax.experimental.pallas.tpu as pltpu

F32 = jnp.float32
BF16 = jnp.bfloat16
U32 = jnp.uint32

B, T, D, U = 2, 4000, 256, 8
QV = T // 8
STEPS = ((0, 128), (128, 128), (256, 128), (384, 120))
NS = len(STEPS)
QP = STEPS[-1][0] + STEPS[-1][1]
NQ = max(n for _, n in STEPS)
XH = 16
JC = 128
NH = 2 * NQ // JC
LASTQ = 64
NSEM = 4

ROUND = ("jt00 jg00 jd00 jz00 df wf jo00 jw00 jt01 jg01 jd01 jz01 d dh c1p c1d w2 jo01 jw01 e w1 "
         "jt10 jg10 jd10 jz10 ah c2d jw10 jo10 jt11 jg11 jd11 jz11 dx jt20 jg20 jd20 jz20 af fe "
         "jo11 jw11 jo20 jw20 jt21 jg21 jd21 jz21 jo21 jt30 jo30 jg30 jd30 jz30 jw21 jt31 jo31 "
         "jw30 jg31 jd31 jz31 jw31 jend")
START = ("NX0/X1 c1p.0 NW1/W2 d1 c1d.0 NX1/X2,WO c1p.1 c1d.1 NW2/G0 ah.0 d2 ah.1 c2d.0 "
         "NX2,WO/X3,G1 Po ge af.0 c1p.2 fe.0 c1d.2 ah.2 c2d.1 NG0/X4 J00.0 af.1 J01.0 fe.1 "
         "NX3/G2,X5 c1p.3 J10.0 c1d.3 ah.3 Pk J11.0 J20.0 c2d.2 J21.0 af.2 J31.0 J30.0 fe.2 "
         "jend.0")
TAIL = "df wf d dh w2 f2 e w1 f1 p1 | p0"

_C0 = 0.7978845608028654
_C1 = 0.044715

W10, W11, W12, W20, W21, W22, WF, WG, WO, W1S, W1D, W2S, W2D = range(13)
A21, A22, A23, A2E, AF = range(5)
AO, A11, A12, A13, A1E = range(5)
_WFORMS = ((WO, False), (WO, True), (W11, True), (W12, True), (W1D, True), (W10, True))


def _nn(a, b):
    return jnp.dot(a, b, preferred_element_type=F32)


def _nt(a, b):
    return jax.lax.dot_general(a, b, (((1,), (1,)), ((), ())), preferred_element_type=F32)


def _tn(a, b):
    return jax.lax.dot_general(a, b, (((0,), (0,)), ((), ())), preferred_element_type=F32)


def _rows(*xs):
    return jnp.concatenate(xs, axis=0)


def _cols(*xs):
    return jnp.concatenate(xs, axis=1)


def _bf(x):
    return x.astype(BF16)


_LEFT = ("11+22", "21+22", "11", "22", "11+12", "21-11", "12-22")
_RIGHT = ("11+22", "11", "12-22", "21-11", "22", "11+12", "21+22")
_LEFT_T = ("11+22", "12+22", "11", "22", "11+21", "12-11", "21-22")
_RIGHT_T = ("11+22", "11", "21-22", "12-11", "22", "11+21", "12+22")
_ORDER = (1, 3, 2, 4, 0, 5, 6)


def _combo(blocks, name):
    if len(name) == 2:
        return blocks[name]
    a, b = blocks[name[:2]], blocks[name[3:]]
    return a + b if name[2] == "+" else a - b


def _str_out(m):
    m1, m2, m3, m4, m5, m6, m7 = m
    return (m4 - m5) + m1 + m7, m3 + m5, m2 + m4, (m3 - m2) + m1 + m6


class _Op:
    def __init__(self, top, bottom=None):
        self.top, self.bottom = top, bottom
        self.cache = {}

    def full(self):
        if "full" not in self.cache:
            self.cache["full"] = _bf(self.top if self.bottom is None
                                     else _rows(self.top, self.bottom))
        return self.cache["full"]

    def get(self, name):
        if name not in self.cache:
            blocks = {"11": self.top[:, :128], "12": self.top[:, 128:],
                      "21": self.bottom[:, :128], "22": self.bottom[:, 128:]}
            self.cache[name] = _bf(_combo(blocks, name))
        return self.cache[name]


def _gelu_and_grad(x):
    w = _C0 + (_C0 * _C1) * (x * x)
    p = 0.5 + 0.5 * jnp.tanh(x * w)
    y = x * p
    g = p + (y * (1.0 - p)) * (6.0 * w - 4.0 * _C0)
    return y, g


def _lo(w):
    return pltpu.unpack_elementwise(w, index=0, packed_dtype=BF16, unpacked_dtype=F32)


def _hi(w):
    return pltpu.unpack_elementwise(w, index=1, packed_dtype=BF16, unpacked_dtype=F32)


def _ld(ref, idx, rows=slice(None)):
    return _cols(*[ref[idx + (c, rows, slice(None))] for c in range(2)])


def _st(ref, idx, rows, val):
    for c in range(2):
        ref[idx + (c, rows, slice(None))] = val[:, c * 128:(c + 1) * 128]


def _ldb(ref, idx):
    return pltpu.bitcast(_cols(*[ref.at[idx + (c,)].bitcast(U32)[...] for c in range(2)]), BF16)


def _stb(ref, idx, val):
    w = pltpu.bitcast(val, U32)
    for c in range(2):
        ref.at[idx + (c,)].bitcast(U32)[...] = w[:, c * 128:(c + 1) * 128]


def _kernel(x_hbm, w1_hbm, w2_hbm, g_hbm, wf_hbm, wg_hbm, wo_hbm, go_hbm,
            out_hbm, dx_hbm, dw1_hbm, dw2_hbm, dg_hbm, dwf_hbm, dwg_hbm, dwo_hbm,
            xbuf, gobuf, outbuf, dxbuf, wbuf, wder, gbuf, fe2, dfe2, sgh, sgf,
            acc, acc7, wout, dgbuf, wstr, sems):

    def halves(src, dst, sem, to_hbm=False):
        cps = []
        for c in range(2):
            lanes = (slice(None),) * (len(src.shape) - 1) + (pl.ds(c * 128, 128),)
            h, v = src.at[lanes], dst(c)
            cps.append(pltpu.make_async_copy(v, h, sem) if to_hbm
                       else pltpu.make_async_copy(h, v, sem))
        return cps

    def x_copies(sem, b, s):
        q0, nq = STEPS[s]
        r0 = max(8 * q0 - 16, 0)
        n = (T if s == NS - 1 else 8 * (q0 + nq) - 16) - r0
        return halves(x_hbm.at[pl.ds(b * T + r0, n)],
                      lambda c: xbuf.at[b, c, pl.ds(XH + r0, n), :], sem)

    def go_copies(sem, b, s):
        q0, nq = STEPS[s]
        n = 16 * (min(q0 + nq, QV) - q0)
        return halves(go_hbm.at[pl.ds(b * 2 * T + 16 * q0, n)],
                      lambda c: gobuf.at[b, c, pl.ds(16 * q0, n), :], sem)

    def out_copies(sem, b, s):
        q0, nq = STEPS[s]
        n = 16 * (min(q0 + nq, QV) - q0)
        return halves(out_hbm.at[pl.ds(b * 2 * T + 16 * q0, n)],
                      lambda c: outbuf.at[b, c, pl.ds(16 * q0, n), :], sem, to_hbm=True)

    def dx_copies(sem, b, s, part=None):
        q0, nq = STEPS[s]
        if part is not None:
            q0, nq = (q0, LASTQ) if part == 0 else (q0 + LASTQ, nq - LASTQ)
        n = 8 * (min(q0 + nq, QV) - q0)
        return halves(dx_hbm.at[pl.ds(b * T + 8 * q0, n)],
                      lambda c: dxbuf.at[b, c, pl.ds(8 * q0, n), :], sem, to_hbm=True)

    def w_copies(sem, i):
        if i in (W10, W20):
            return halves({W10: w1_hbm, W20: w2_hbm}[i],
                          lambda c: wbuf.at[pl.ds(i, 3), c], sem)
        return halves({WF: wf_hbm, WG: wg_hbm, WO: wo_hbm}[i], lambda c: wbuf.at[i, c], sem)

    def g_copies(sem):
        return halves(g_hbm, lambda c: gbuf.at[c], sem)

    def dw_copies(sem, i):
        dst = {W10: dw1_hbm.at[0], W11: dw1_hbm.at[1], W12: dw1_hbm.at[2], W20: dw2_hbm.at[0],
               W21: dw2_hbm.at[1], W22: dw2_hbm.at[2], WF: dwf_hbm, WG: dwg_hbm, WO: dwo_hbm}[i]
        return halves(dst, lambda c: wout.at[i, c], sem, to_hbm=True)

    def dg_copies(sem):
        return halves(dg_hbm, lambda c: dgbuf.at[c], sem, to_hbm=True)

    order = [(b, s) for b in range(B) for s in reversed(range(NS))]
    makers = {"w": w_copies, "g": g_copies, "x": x_copies, "go": go_copies,
              "out": out_copies, "dx": dx_copies, "dw": dw_copies, "dg": dg_copies}
    X = lambda i: ("x",) + order[i]
    GO = lambda i: ("go",) + order[i]
    OUT = lambda i: ("out",) + order[i]
    DX = lambda i: ("dx",) + order[i]
    W1_ = [("w", W10)]
    W2_ = [("w", W20), ("w", WF)]
    WO_ = [("w", WG), ("g",), ("w", WO)]

    groups = [tuple(g) for g in (
        [X(0)], W1_, [X(1)], W2_, [X(2)] + WO_, [GO(0)], [X(3)], [GO(1), X(4), GO(2), X(5)],
        [GO(3), X(6), GO(4), X(7)], [GO(5), GO(6)], [GO(7)])]
    group_of = {k: g for g in groups for k in g}
    free_slots = list(range(NSEM - 1))
    slot_of = {}
    started = set()
    waited = set()

    def copies(key):
        slot = slot_of[group_of[key]] if key in group_of else NSEM - 1
        return makers[key[0]](sems.at[slot], *key[1:])

    def put(*key):
        assert key not in started
        if key in group_of and group_of[key] not in slot_of:
            slot_of[group_of[key]] = free_slots.pop(0)
        for cp in copies(key):
            cp.start()
        started.add(key)

    def need(*keys, then=()):
        for k in keys:
            assert k in started and k not in waited, k
            assert k not in group_of or all(m in keys for m in group_of[k]), k
        for k in keys:
            for cp in copies(k):
                cp.wait()
            waited.add(k)
        for g in dict.fromkeys(group_of[k] for k in keys if k in group_of):
            free_slots.append(slot_of[g])
        for k in then:
            put(*k)

    for key in [X(0)] + W1_:
        put(*key)

    for b in range(B):
        for c in range(2):
            xbuf[b, c, 0:XH, :] = jnp.zeros((XH, 128), BF16)
            xbuf[b, c, XH + T:XH + 8 * QP, :] = jnp.zeros((8 * QP - T, 128), BF16)
            gobuf[b, c, 2 * T:16 * QP, :] = jnp.zeros((16 * QP - 2 * T, 128), BF16)

    state = {}
    facts = set()
    n_acc = {}

    def W(i):
        if i < 9:
            assert ("w", i - i % 3 if i < WF else i) in waited
            return _ldb(wbuf, (i,))
        assert ("derived", i) in facts
        return pltpu.bitcast(_ld(wder, (i - 9,)), BF16)

    def derive(slot_sum, slot_diff, i0, i2):
        a0, a2 = W(i0).astype(F32), W(i2).astype(F32)
        _st(wder, (slot_sum - 9,), slice(None), pltpu.bitcast(_bf(a0 + a2), U32))
        _st(wder, (slot_diff - 9,), slice(None), pltpu.bitcast(_bf(a0 - a2), U32))
        facts.update([("derived", slot_sum), ("derived", slot_diff)])

    def w_prepare(i, transposed):
        w = W(i).astype(F32)
        blocks = {"11": w[:128, :128], "12": w[:128, 128:], "21": w[128:, :128],
                  "22": w[128:, 128:]}
        for n, name in enumerate(_RIGHT_T if transposed else _RIGHT):
            m = _combo(blocks, name)
            wstr[7 * _WFORMS.index((i, transposed)) + n] = pltpu.bitcast(
                _bf(m.T if transposed else m), U32)
        facts.add(("prepared", i, transposed))

    def strassen(op, i, transposed):
        assert ("prepared", i, transposed) in facts
        m = [None] * 7
        for n in _ORDER:
            w = pltpu.bitcast(wstr[7 * _WFORMS.index((i, transposed)) + n], BF16)
            m[n] = _nn(op.get(_LEFT[n]), w)
        return _str_out(m)

    def mm_s(op, i, transposed):
        c11, c12, c21, c22 = strassen(op, i, transposed)
        return _cols(c11, c12), _cols(c21, c22)

    def mm(op, i, transposed=False):
        y = (_nt if transposed else _nn)(op.full(), W(i))
        if op.bottom is None:
            return y
        n = op.top.shape[0]
        return y[:n], y[n:]

    def accumulate(slot, a, d):
        val = _tn(a.full(), d.full())
        acc[slot] = acc[slot] + val if ("n", slot) in n_acc else val
        n_acc["n", slot] = n_acc.get(("n", slot), 0) + 1

    def accumulate_s(slot, a, d):
        for n in _ORDER:
            val = _tn(d.get(_LEFT_T[n]), a.get(_RIGHT[n]))
            k = 7 * slot + n
            acc7[k] = acc7[k] + val if ("s", slot) in n_acc else val
        n_acc["s", slot] = n_acc.get(("s", slot), 0) + 1

    def accumulated(slot):
        assert n_acc["n", slot] == B * NS
        return acc[slot]

    def accumulated_s(slot):
        assert n_acc["s", slot] == B * NS * {AO: 4 * NH, A1E: 2}.get(slot, 1)
        c11, c12, c21, c22 = _str_out([acc7[7 * slot + n] for n in range(7)])
        return _rows(_cols(c11, c12), _cols(c21, c22)).T

    def conv1_operands(b, s):
        q0, nq = STEPS[s]
        assert ("x", b, s) in waited and (s == NS - 1 or ("x", b, s + 1) in waited)

        def words(j):
            start_row = XH // 2 + 4 * q0 + j
            return _cols(*[xbuf.at[b, c].bitcast(U32)[pl.ds(start_row, nq, stride=4), :]
                           for c in range(2)])

        xs = []
        for j in range(4):
            w = words(j)
            xs += [_lo(w), _hi(w)]
        x7s = _hi(words(-1))
        return (_Op(x7s - xs[1], xs[3] - xs[5]), _Op(xs[1], xs[5]),
                _Op(xs[3] - xs[1], xs[7] - xs[5]), _Op(xs[0], xs[4]), _Op(xs[2], xs[6]))

    def conv1_prep(b, s):
        state["x", b, s] = conv1_operands(b, s)

    def conv1_dots(b, s):
        q0, nq = STEPS[s]
        x1, x2, x3, xa, xb = state.pop(("x", b, s))
        e = _nn(_bf(_rows(xa.top, xa.bottom, xb.top, xb.bottom)), W(W11))
        ea, eb = (e[:nq], e[nq:2 * nq]), (e[2 * nq:3 * nq], e[3 * nq:])
        m1 = mm(x1, W10)
        m3 = mm(x3, W12)
        m2 = mm(x2, W1S)
        state["hp", b, s] = [m1[0] + m2[0] + ea[0], m2[0] + m3[0] + eb[0],
                             m1[1] + m2[1] + ea[1], m2[1] + m3[1] + eb[1]]

    def act_h(b, s):
        q0, nq = STEPS[s]
        hp = state.pop(("hp", b, s))
        h = []
        for a in range(4):
            y, gr = _gelu_and_grad(hp[a])
            h.append(y)
            sgh[b, s, a, 0:nq, :] = gr
        state["h3_last", b, s] = h[3][nq - 1:nq]
        d31 = _rows(jnp.zeros((1, D), F32), h[3][:nq - 1]) - h[1]
        state["hpart", b, s] = (d31, _Op(h[1]), _Op(h[3] - h[1]), _Op(h[0], h[2]))

    def conv2_dots(b, s):
        d31, h2, h3, he = state.pop(("hpart", b, s))
        if s > 0:
            first = jax.lax.broadcasted_iota(jnp.int32, (8, D), 0) == 0
            below = jnp.broadcast_to(state.pop(("h3_last", b, s - 1)), (8, D))
            d31 = _rows(jnp.where(first, d31[:8] + below, d31[:8]), d31[8:])
        h1 = _Op(d31)
        e = mm(he, W21)
        m3 = mm(h3, W22)
        m2 = mm(h2, W2S)
        m1 = mm(h1, W20)
        state["h", b, s] = (h1, h2, h3, he)
        state["fp", b, s] = [m1 + m2 + e[0], m2 + m3 + e[1]]

    def act_f(b, s):
        q0, nq = STEPS[s]
        fp = state.pop(("fp", b, s))
        f = []
        for c in range(2):
            y, gr = _gelu_and_grad(fp[c])
            f.append(y)
            sgf[b, s, c, 0:nq, :] = gr
        state["f", b, s] = _Op(f[0], f[1])

    def fe_dots(b, s):
        q0, nq = STEPS[s]
        fe = mm(state["f", b, s], WF)
        for c in range(2):
            _st(fe2, (b,), pl.ds(2 * q0 + c, nq, stride=2), fe[c])
        facts.add(("fe", b, s))

    def ge_setup():
        assert ("g",) in waited
        ge = _nn(_ldb(gbuf, ()), W(WG))
        state["ge"] = [jnp.broadcast_to(ge[r:r + 1], (8, D)) for r in range(B * U)]
        state["dge"] = {}

    def chunk(s, h):
        nt = 2 * STEPS[s][1]
        return h * JC, min(JC, nt - h * JC)

    def tanh_pair(b, s, k, h):
        q0, nq = STEPS[s]
        assert ("fe", b, s) in facts
        r0, n = chunk(s, h)
        fe = _ld(fe2, (b,), slice(2 * q0 + r0, 2 * q0 + r0 + n)).reshape(n // 8, 8, D)
        return [jnp.tanh((fe + state["ge"][b * U + 2 * k + p][None]).reshape(n, D))
                for p in range(2)]

    def j_tanh(b, s, k, h):
        state["j", b, s, k, h] = _Op(*tanh_pair(b, s, k, h))

    def j_g(b, s, k, h):
        q0, nq = STEPS[s]
        assert ("go", b, s) in waited
        r0, n = chunk(s, h)
        gw = _cols(*[gobuf.at[b, c].bitcast(U32)[pl.ds(8 * q0 + 4 * r0 + k, n, stride=4), :]
                     for c in range(2)])
        state["g", b, s, k, h] = _Op(_lo(gw), _hi(gw))

    def j_dj(b, s, k, h):
        state["dj", b, s, k, h] = strassen(state["g", b, s, k, h], WO, True)

    def j_out(b, s, k, h):
        q0, nq = STEPS[s]
        r0, n = chunk(s, h)
        c11, c12, c21, c22 = strassen(state["j", b, s, k, h], WO, False)
        for c, (lo, hi) in enumerate(((c11, c21), (c12, c22))):
            outbuf.at[b, c].bitcast(U32)[pl.ds(8 * q0 + 4 * r0 + k, n, stride=4), :] = (
                pltpu.pack_elementwise([lo, hi], packed_dtype=BF16))
        facts.add(("out", b, s, k, h))

    def j_dz(b, s, k, h):
        r0, n = chunk(s, h)
        jp = tanh_pair(b, s, k, h)
        d11, d12, d21, d22 = state.pop(("dj", b, s, k, h))
        dz = [dj * (1.0 - j * j) for dj, j in zip((_cols(d11, d12), _cols(d21, d22)), jp)]
        both = dz[0] + dz[1]
        key = ("dsum", b, s, h)
        assert ("dz", b, s, k - 1, h) in facts or k == 0
        facts.add(("dz", b, s, k, h))
        state[key] = both if k == 0 else state[key] + both
        for p in range(2):
            part = jnp.sum(dz[p].reshape(n // 8, 8, D), axis=0)
            key = b * U + 2 * k + p
            state["dge"][key] = part + state["dge"][key] if key in state["dge"] else part

    def j_dwo(b, s, k, h):
        accumulate_s(AO, state["j", b, s, k, h], state["g", b, s, k, h])

    def joint_end(b, s):
        q0, nq = STEPS[s]
        assert all((n, b, s, k, h) in facts for n in ("out", "dz") for k in range(4)
                   for h in range(NH))
        put("out", b, s)
        slot = (b * NS + s) % 2
        for h in range(NH):
            r0, n = chunk(s, h)
            _st(dfe2, (slot,), slice(r0, r0 + n), state.pop(("dsum", b, s, h)))
        state["dfe", b, s] = _Op(*[_ld(dfe2, (slot,), pl.ds(c, nq, stride=2)) for c in range(2)])

    def bwd_df(b, s):
        state["df", b, s] = mm(state["dfe", b, s], WF, True)

    def bwd_wf(b, s):
        accumulate(AF, state["f", b, s], state["dfe", b, s])

    def bwd_d(b, s):
        q0, nq = STEPS[s]
        df = state.pop(("df", b, s))
        d0 = df[0] * sgf[b, s, 0, 0:nq, :]
        d1 = df[1] * sgf[b, s, 1, 0:nq, :]
        nxt = jnp.zeros((1, D), F32) if s == NS - 1 else state["d0_first"]
        state["d0_first"] = d0[0:1]
        d0s = _rows(d0[1:], nxt)
        state["d", b, s] = (_Op(d0, d1), _Op(d0), _Op(d1), _Op(d0 + d1), _Op(d1 + d0s))

    def bwd_h(b, s):
        q0, nq = STEPS[s]
        de, d0, d1, s01, s10 = state["d", b, s]
        dhe = mm(de, W21, True)
        n1 = mm(s01, W22, True)
        n3 = mm(s10, W20, True)
        n2 = mm(d1, W2D, True)
        dh = [dhe[0], n1 + n2, dhe[1], n3 - n2]
        e = [dh[a] * sgh[b, s, a, 0:nq, :] for a in range(4)]
        nxt = jnp.zeros((1, D), F32) if s == NS - 1 else state["e0_first"]
        state["e0_first"] = e[0][0:1]
        state["e32", b, s] = e + [_rows(e[0][1:], nxt)]

    def e_operands(e32, rows=slice(None)):
        e0, e1, e2, e3, e0s = [v[rows] for v in e32]
        return (_Op(e0, e2), _Op(e0 + e1, e2 + e3), _Op(e1, e3), _Op(e1 + e2, e3 + e0s))

    def bwd_e(b, s):
        state["e", b, s] = e_operands(state["e32", b, s])

    def bwd_w2(b, s):
        de, d0, d1, s01, s10 = state["d", b, s]
        h1, h2, h3, he = state["h", b, s]
        accumulate(A21, h1, d0)
        accumulate(A22, h2, s01)
        accumulate(A23, h3, d1)
        accumulate(A2E, he, de)

    def bwd_w1(b, s):
        e1, e2, e3, e4 = state["e", b, s]
        x1, x2, x3, xa, xb = conv1_operands(b, s)
        accumulate_s(A11, x1, e1)
        accumulate_s(A12, x2, e2)
        accumulate_s(A13, x3, e3)
        accumulate_s(A1E, xa, e1)
        accumulate_s(A1E, xb, e3)

    def dx_dots(b, s, ops, q0, nq):
        e1, e2, e3, e4 = ops
        dxa, dxb = mm_s(e1, W11, True), mm_s(e3, W11, True)
        n1 = mm_s(e2, W12, True)
        n2 = mm_s(e3, W1D, True)
        n3 = mm_s(e4, W10, True)
        dx = [dxa[0], n1[0] + n2[0], dxb[0], n3[0] - n2[0],
              dxa[1], n1[1] + n2[1], dxb[1], n3[1] - n2[1]]
        for j in range(4):
            w = pltpu.pack_elementwise([dx[2 * j], dx[2 * j + 1]], packed_dtype=BF16)
            for c in range(2):
                dxbuf.at[b, c].bitcast(U32)[pl.ds(4 * q0 + j, nq, stride=4), :] = (
                    w[:, c * 128:(c + 1) * 128])

    def bwd_dx(b, s):
        q0, nq = STEPS[s]
        dx_dots(b, s, state["e", b, s], q0, nq)
        put("dx", b, s)

    def bwd_dx_part(b, s, part):
        q0, nq = STEPS[s]
        r0, nq = (0, LASTQ) if part == 0 else (LASTQ, nq - LASTQ)
        dx_dots(b, s, e_operands(state["e32", b, s], slice(r0, r0 + nq)), q0 + r0, nq)
        put("dx", b, s, part)

    def put_w(i, *vals):
        for n, val in enumerate(vals):
            _stb(wout, (i + n,), _bf(val))
            put("dw", i + n)

    def finish_w1():
        a2 = accumulated_s(A12)
        put_w(W10, accumulated_s(A11) + a2, accumulated_s(A1E), a2 + accumulated_s(A13))

    def finish_w2():
        a2 = accumulated(A22)
        put_w(W20, accumulated(A21) + a2, accumulated(A2E), a2 + accumulated(A23))
        put_w(WF, accumulated(AF))

    def finish_g():
        assert len(state["dge"]) == B * U
        dge = _bf(_rows(*[jnp.sum(state["dge"][r], axis=0, keepdims=True)
                          for r in range(B * U)]))
        _stb(dgbuf, (), _bf(_nt(dge, W(WG))))
        put("dg")
        put_w(WG, _tn(_ldb(gbuf, ()), dge))

    atoms = {"df": ("k", bwd_df), "wf": ("k", bwd_wf), "d": ("k", bwd_d), "dh": ("k", bwd_h),
             "w2": ("k", bwd_w2), "e": ("k", bwd_e), "w1": ("k", bwd_w1), "dx": ("k", bwd_dx),
             "c1p": ("c1", conv1_prep), "c1d": ("c1", conv1_dots), "ah": ("c1", act_h),
             "c2d": ("c2", conv2_dots), "af": ("c2", act_f), "fe": ("c2", fe_dots),
             "jend": ("j", joint_end)}
    for k in range(4):
        for h in range(NH):
            for nm, fn in (("jt", j_tanh), ("jg", j_g), ("jd", j_dj), ("jo", j_out),
                           ("jz", j_dz), ("jw", j_dwo)):
                atoms["%s%d%d" % (nm, k, h)] = (
                    "j", lambda b, s, fn=fn, k=k, h=h: fn(b, s, k, h))

    def round_(c1=None, c2=None, jb=None, kb=None, seq=ROUND, fence=None):
        steps = {"c1": c1, "c2": c2, "j": jb, "k": kb}
        for name in seq.split():
            if fence is not None and name == fence[0]:
                fence[1]()
            who, fn = atoms[name]
            if steps[who] is not None:
                fn(*steps[who])

    o = order
    weight_sets = {"W1": W1_, "W2": W2_, "WO": WO_}
    forms = {"o": _WFORMS[:2], "k": _WFORMS[2:]}

    def keys(spec):
        out = []
        for t in spec.split(","):
            if t in weight_sets:
                out += weight_sets[t]
            elif t:
                out.append((X if t[0] == "X" else GO)(int(t[1:])))
        return out

    for tok in START.split():
        if tok[0] == "N":
            wanted, then = tok[1:].split("/")
            need(*keys(wanted), then=keys(then))
        elif tok == "d1":
            derive(W1S, W1D, W10, W12)
        elif tok == "d2":
            derive(W2S, W2D, W20, W22)
        elif tok == "ge":
            ge_setup()
        elif tok[0] == "P":
            for form in forms[tok[1]]:
                w_prepare(*form)
        else:
            name, i = tok.split(".")
            seq = " ".join(x + name[1:] for x in ("jt", "jg", "jd", "jz", "jo", "jw")) \
                if name[0] == "J" else name
            step = o[int(i)]
            round_(c1=step, c2=step, jb=step, kb=step, seq=seq)

    need(GO(1), X(4), GO(2), X(5), then=[GO(3), X(6), GO(4), X(7)])
    round_(c1=o[4], c2=o[3], jb=o[1], kb=o[0])
    round_(c1=o[5], c2=o[4], jb=o[2], kb=o[1], fence=(
        "jt30", lambda: need(GO(3), X(6), GO(4), X(7), then=[GO(5), GO(6), GO(7)])))
    round_(c1=o[6], c2=o[5], jb=o[3], kb=o[2])
    round_(c1=o[7], c2=o[6], jb=o[4], kb=o[3], fence=(
        "jend", lambda: need(GO(5), GO(6), OUT(0), OUT(1), DX(0))))
    round_(c2=o[7], jb=o[5], kb=o[4])
    round_(jb=o[6], kb=o[5], fence=("jend", lambda: need(GO(7), DX(1))))
    round_(jb=o[7], kb=o[6])
    finish_g()
    put_w(WO, accumulated_s(AO))
    need(OUT(2), OUT(3), OUT(4), OUT(5), DX(2), DX(3), DX(4))
    tail = {"f2": finish_w2, "f1": finish_w1, "p0": lambda: bwd_dx_part(*o[7], 0),
            "p1": lambda: bwd_dx_part(*o[7], 1), "|": lambda: need(OUT(6), DX(5))}
    for name in TAIL.split():
        if name in tail:
            tail[name]()
        else:
            round_(kb=o[7], seq=name)

    for key in sorted(started - waited, key=str):
        need(key)


@jax.jit
def pallas_standalone__seq2seq_rnn_t_joint__speech_kernel(
    x: jax.Array,
    w1: jax.Array,
    w2: jax.Array,
    g: jax.Array,
    w_f: jax.Array,
    w_g: jax.Array,
    w_o: jax.Array,
    grad_out: jax.Array,
):
    hbm = pl.BlockSpec(memory_space=pl.ANY)
    out_shape = (
        jax.ShapeDtypeStruct((B * 2 * T, D), BF16),
        jax.ShapeDtypeStruct((B * T, D), BF16),
        jax.ShapeDtypeStruct((3, D, D), BF16),
        jax.ShapeDtypeStruct((3, D, D), BF16),
        jax.ShapeDtypeStruct((B * U, D), BF16),
        jax.ShapeDtypeStruct((D, D), BF16),
        jax.ShapeDtypeStruct((D, D), BF16),
        jax.ShapeDtypeStruct((D, D), BF16),
    )
    scratch = [
        pltpu.VMEM((B, 2, XH + 8 * QP, 128), BF16),
        pltpu.VMEM((B, 2, 16 * QP, 128), BF16),
        pltpu.VMEM((B, 2, 16 * QP, 128), BF16),
        pltpu.VMEM((B, 2, 8 * QP, 128), BF16),
        pltpu.VMEM((9, 2, D, 128), BF16),
        pltpu.VMEM((4, 2, D // 2, 128), U32),
        pltpu.VMEM((2, B * U, 128), BF16),
        pltpu.VMEM((B, 2, 2 * QP, 128), F32),
        pltpu.VMEM((2, 2, 2 * NQ, 128), F32),
        pltpu.VMEM((B, NS, 4, NQ, D), F32),
        pltpu.VMEM((B, NS, 2, NQ, D), F32),
        pltpu.VMEM((5, D, D), F32),
        pltpu.VMEM((7 * 5, 128, 128), F32),
        pltpu.VMEM((9, 2, D, 128), BF16),
        pltpu.VMEM((2, B * U, 128), BF16),
        pltpu.VMEM((7 * len(_WFORMS), 64, 128), U32),
        pltpu.SemaphoreType.DMA((NSEM,)),
    ]
    out, dx, dw1, dw2, dg, dwf, dwg, dwo = pl.pallas_call(
        _kernel,
        out_shape=out_shape,
        in_specs=[hbm] * 8,
        out_specs=tuple([hbm] * 8),
        scratch_shapes=scratch,
        compiler_params=pltpu.CompilerParams(vmem_limit_bytes=110 * 2**20),
        name="rnnt_joint_fwd_bwd",
    )(x.reshape(B * T, D), w1, w2, g.reshape(B * U, D), w_f, w_g, w_o,
      grad_out.reshape(B * 2 * T, D))
    return (out.reshape(B, T // 4, U, D), dx.reshape(B, T, D), dw1, dw2, dg.reshape(B, U, D),
            dwf, dwg, dwo)
```
